```python
import os as _os
_os.environ.setdefault("JAX_PLATFORMS", "cpu")
import jax
import jax.numpy as jnp

def _softmax(x, axis=-1):
    return jax.nn.softmax(x, axis=axis)
def _gelu(x):
    return jax.nn.gelu(x, approximate=True)
def _silu(x):
    return jax.nn.silu(x)
def _sigmoid(x):
    return jax.nn.sigmoid(x)
def _layernorm(x, axis=-1, eps=1e-5):
    m = jnp.mean(x, axis=axis, keepdims=True)
    v = jnp.var(x, axis=axis, keepdims=True)
    return (x - m) / jnp.sqrt(v + eps)
def _scatter_add(tgt, idx, src, axis=0):
    return tgt.at[idx].add(src)
def _segment_sum(src, seg, n):
    return jax.ops.segment_sum(src, seg, n)
class _Rng:
    def __init__(self, key):
        self._k = key
    def _next(self):
        self._k, sub = jax.random.split(self._k)
        return sub
    def normal(self, shape):
        return jax.random.normal(self._next(), shape, dtype=jnp.bfloat16)
    def randint(self, lo, hi, shape):
        return jax.random.randint(self._next(), shape, lo, hi, dtype=jnp.int32)
    def uniform(self, shape, lo=0.0, hi=1.0):
        return jax.random.uniform(self._next(), shape, jnp.bfloat16, lo, hi)
    def permutation(self, n):
        return jax.random.permutation(self._next(), n)


kernel_name = 'sequential_preLN__sliding_block__swiglu_ffn__prompt'

def setup_inputs():
    _rng = _Rng(jax.random.key(int.from_bytes(__import__("os").urandom(4), "little")))
    _w = (lambda a: (lambda t: t.astype(jnp.bfloat16) if jnp.issubdtype(t.dtype, jnp.floating) else t)(jnp.asarray(a)))
    def _A_setup():
        B, S, D = 1, 2048, 512
        return {
            "x": _w((lambda *s: _rng.normal(s) * 0.05)(B, S, D)),
            "wqkv": _w((lambda *s: _rng.normal(s) * 0.05)(D, 3 * D)),
            "wo": _w((lambda *s: _rng.normal(s) * 0.05)(D, D)),
        }
    _A_in = _A_setup()

    def _B_setup():
        B, S, D, F = 1, 2048, 512, 1792
        return {
            "x": _w((lambda *s: _rng.normal(s) * 0.05)(B, S, D)),
            "w_gate": _w((lambda *s: _rng.normal(s) * 0.05)(D, F)),
            "w_up": _w((lambda *s: _rng.normal(s) * 0.05)(D, F)),
            "w_down": _w((lambda *s: _rng.normal(s) * 0.05)(F, D)),
        }
    _B_in = _B_setup()

    return {
        "A_x": _A_in["x"],
        "A_wqkv": _A_in["wqkv"],
        "A_wo": _A_in["wo"],
        "B_x": _B_in["x"],
        "B_w_gate": _B_in["w_gate"],
        "B_w_up": _B_in["w_up"],
        "B_w_down": _B_in["w_down"],
    }

def reference(A_x, A_wqkv, A_wo, B_x, B_w_gate, B_w_up, B_w_down):
    def _A_ref(x, wqkv, wo):
        B, S, D = x.shape
        H = 32; Dh = D // H; W = 256
        qkv = (lambda x, *d: x.transpose(*d))((x @ wqkv).reshape(B, S, 3, H, Dh), 2, 0, 3, 1, 4)
        q, k, v = qkv[0], qkv[1], qkv[2]
        scores = jnp.einsum("bhqd,bhkd->bhqk", q, k) * (Dh ** -0.5)
        idx = jnp.arange(S)
        mask = (idx[:, None] - idx[None, :] >= 0) & (idx[:, None] - idx[None, :] < W)
        scores = jnp.where(mask[None, None], scores, -1e9)
        p = _softmax(scores, axis=-1)
        o = jnp.einsum("bhqk,bhkd->bhqd", p, v)
        return (lambda x, *d: x.transpose(*d))(o, 0, 2, 1, 3).reshape(B, S, D) @ wo

    def _B_ref(x, w_gate, w_up, w_down):
        g = _silu(x @ w_gate)
        u = x @ w_up
        return (g * u) @ w_down

    x = A_x
    h = x + _A_ref(_layernorm(x, axis=-1), A_wqkv, A_wo)
    h2 = h + _B_ref(_layernorm(h, axis=-1), B_w_gate, B_w_up, B_w_down)
    return h2
```

```python
import functools
import math

import jax
import jax.numpy as jnp
from jax import lax
import jax.experimental.pallas as pl
import jax.experimental.pallas.tpu as pltpu

DH = 16
W = 256
LANES = 128
QBLK = 128
EPS = 1e-5
BF16 = jnp.bfloat16
F32 = jnp.float32
U32 = jnp.uint32
NT = (((1,), (1,)), ((), ()))


def _bits(x):
    return pltpu.bitcast(x, U32)


def _bf16(x):
    return pltpu.bitcast(x, BF16)


def _pack(x):
    return jnp.concatenate(
        [pltpu.pack_elementwise([x[r:r + 8], x[r + 8:r + 16]], packed_dtype=BF16).astype(U32)
         for r in range(0, x.shape[0], 16)], axis=0)


def _unpack(w):
    return jnp.concatenate(
        [pltpu.unpack_elementwise(w[r:r + 8], index=k, packed_dtype=BF16, unpacked_dtype=F32)
         for r in range(0, w.shape[0], 8) for k in range(2)], axis=0)


def _dot(a, b):
    return jnp.dot(a, b, preferred_element_type=F32)


def _layernorm(x):
    m = jnp.mean(x, axis=-1, keepdims=True)
    c = x - m
    v = jnp.mean(c * c, axis=-1, keepdims=True)
    return c * lax.rsqrt(v + EPS)


def _sel(mask, a, b):
    if a is None and b is None:
        return None
    if a is None:
        a = jnp.zeros_like(b)
    if b is None:
        b = jnp.zeros_like(a)
    return jnp.where(mask, a, b)


def _ds(start, size, align):
    if isinstance(start, int):
        return pl.ds(start, size)
    return pl.ds(pl.multiple_of(start, align), size)


def _scores(q_ref, k_ref, tok0, skip, slab, G, which):
    QB = QBLK // G
    a = QB // 16
    lanes = pl.ds(slab * LANES, LANES)
    qlane = lax.broadcasted_iota(jnp.int32, (QB // 2, LANES), 1) // DH
    half0 = tok0 // 2
    sts = []
    for u in range(8 // G):
        for s in range(G):
            if u * G + s not in which:
                continue
            qs = q_ref[_ds(half0 + s * QB // 2, QB // 2, 8), lanes]
            qbd = _bf16(jnp.concatenate(
                [jnp.where(qlane == u * G + (p ^ s), qs, jnp.zeros_like(qs)) for p in range(G)], axis=0))
            lo = max(s * a, skip)
            hi = s * a + 16 + a
            kwin = _bf16(k_ref[_ds(half0 - W // 2 + 8 * lo, 8 * (hi - lo), 8), lanes])
            sts.append(lax.dot_general(kwin, qbd, NT, preferred_element_type=F32))
    return sts


def _edge_mask(G):
    QB = QBLK // G
    er = lax.broadcasted_iota(jnp.int32, (QB, LANES), 0)
    ei = lax.broadcasted_iota(jnp.int32, (QB, LANES), 1) & (QB - 1)
    return er > ei


def _merge(st, skip, s, G, s_ref):
    QB = QBLK // G
    a = QB // 16
    n = st.shape[0]
    last = st[n - QB:]
    if s * a >= skip:
        parts = [st[QB:n - QB], jnp.where(_edge_mask(G), st[:QB], last)]
    else:
        parts = [st[:n - QB]] if n > QB else []
        parts.append(jnp.where(_edge_mask(G), -1e30, last))
    sm = jnp.concatenate(parts, axis=0)
    m = jnp.max(sm, axis=0, keepdims=True)
    if s_ref is None:
        return (lambda: sm), m
    rows = pl.ds(0, sm.shape[0])
    s_ref[rows, :] = sm
    return (lambda: s_ref[rows, :]), m


def _softmax(scores, skip, s, G, GPV, p_ref):
    QB = QBLK // G
    a = QB // 16
    old = _edge_mask(G)
    lo = max(s * a, skip)
    hi = s * a + 16 + a
    sm, m = scores[0](), scores[1]
    nm = sm.shape[0] - QB
    pf = jnp.exp2(sm - m)
    total = jnp.broadcast_to(jnp.sum(pf, axis=0, keepdims=True), (8, LANES)) if GPV == 2 else None
    pe = pf[nm:]
    parts = [jnp.where(old, pe, 0.0)] if lo == s * a else []
    parts += [pf[:nm]] if nm else []
    parts += [jnp.where(old, 0.0, pe)]
    packed = _pack(jnp.concatenate(parts, axis=0))
    if p_ref is not None:
        p_ref[pl.ds(0, packed.shape[0]), :] = packed
        get = lambda j: p_ref[pl.ds(8 * j, 8), :]
    else:
        get = lambda j: packed[8 * j:8 * j + 8]
    return (lo, hi, get), total


def _unskew(tiles, t, skip, G, GPV):
    QB = QBLK // G
    lane = lax.broadcasted_iota(jnp.int32, (8, LANES), 1)
    nst = int(math.log2(G)) - (GPV - 1)

    def pick(t, k, w):
        if k == 0:
            lo, hi, get = tiles[t]
            return get(w - lo) if lo <= w < hi else None
        bit = ((lane // QB) >> (k - 1)) & 1 == 1
        return _sel(bit, pick(t ^ (1 << (k - 1)), k - 1, w), pick(t, k - 1, w))
    rows = [pick(t, nst, w) for w in range(skip // 8 * 8, 24)]
    return _bf16(jnp.concatenate([x if x is not None else jnp.zeros((8, LANES), U32) for x in rows], axis=0))


def _pv(pt, vt_ref, tok0, skip, slab, h, G, GPV):
    w0 = skip // 8 * 8
    nk = 16 * (24 - w0)
    kcols = _ds(tok0 - W + 16 * w0, nk, LANES)
    v0 = vt_ref[pl.ds((slab * 8 + h) * 8, 8), kcols]
    if GPV == 1:
        v1 = jnp.full((8, nk), 0x3F803F80, U32)
    else:
        v1 = vt_ref[pl.ds((slab * 8 + (h ^ (G // 2))) * 8, 8), kcols]
    return _dot(_bf16(jnp.concatenate([v0, v1], axis=0)), pt)


def _finish(res, rs, o_ref, tok0, slab, G, GPV):
    lane = lax.broadcasted_iota(jnp.int32, (8, LANES), 1)
    outs = []
    if GPV == 2:
        for k in range(int(math.log2(G))):
            bit = ((lane // (QBLK // G)) >> k) & 1 == 1
            rs = [jnp.where(bit, rs[t ^ (1 << k)], rs[t]) for t in range(8)]
        rs = [1.0 / x for x in rs]
    for h in range(8):
        if GPV == 1:
            r = 1.0 / res[h][16:24]
            outs += [res[h][:8] * r, res[h][8:16] * r]
        else:
            o2 = res[h ^ (G // 2)]
            outs += [jnp.where(lane < 64, res[h][:8], o2[16:24]) * rs[h],
                     jnp.where(lane < 64, res[h][8:16], o2[24:]) * rs[h]]
    o = _bits(jnp.concatenate(outs, axis=0).astype(BF16).T)
    n = QBLK // G // 2
    hl = lax.broadcasted_iota(jnp.int32, (n, LANES), 1) // DH
    parts = [o[p * n:(p + 1) * n] for p in range(G)]
    for k in range(int(math.log2(G))):
        bit = (hl >> k) & 1 == 1
        parts = [jnp.where(bit, parts[t ^ (1 << k)], parts[t]) for t in range(G)]
    o_ref[_ds(tok0 // 2, QBLK // 2, 8), pl.ds(slab * LANES, LANES)] = jnp.concatenate(parts, axis=0)


def _behind(words, after):
    if after is None:
        return words
    lane = lax.broadcasted_iota(jnp.int32, words.shape, 1)
    never = (lane * lane) & 2 != 0
    anchor = jnp.concatenate([pltpu.bitcast(after[:8], U32)] * (words.shape[1] // LANES), axis=1)
    return jnp.where(never, anchor, words)


def _lhs_operands(a11, a12, a21, a22):
    return [a11 + a22, a21 + a22, a11, a22, a11 + a12, a21 - a11, a12 - a22]


def _rhs_operands(b11, b12, b21, b22):
    return [b11 + b22, b11, b12 - b22, b21 - b11, b22, b11 + b12, b21 + b22]


def _combine(m):
    return (m[0] + m[3]) + (m[6] - m[4]), m[2] + m[4], m[1] + m[3], (m[0] - m[1]) + (m[2] + m[5])


def _kernel(x_hbm, wqkv_hbm, wo_hbm, wg_hbm, wu_hbm, wd_hbm, out_hbm,
            x_ref, wqkv_ref, wo_ref, wg_ref, wu_ref, wd_ref, out_ref,
            xn_ref, q_ref, k_ref, vt_ref, o_ref, h_ref, hn_ref, a_ref, sg_ref, su_ref, sd_ref, p_ref, y_ref, s_ref, xs_ref, sq_ref, in_sems, out_sems,
            *, TB, G, GPV, NP, NS, NG, program):
    S, D = out_ref.shape
    F = wg_ref.shape[-1]
    NB = S // TB
    scale = DH ** -0.5 * math.log2(math.e)

    def in_copy(n, src, dst):
        return pltpu.make_async_copy(src, dst, in_sems.at[n])

    x_hbm, wqkv_hbm, wo_hbm, wg_hbm, wu_hbm, wd_hbm = (r.bitcast(U32) for r in (x_hbm, wqkv_hbm, wo_hbm, wg_hbm, wu_hbm, wd_hbm))
    first = pl.ds(0, TB // 2)
    rest = pl.ds(TB // 2, (S - TB) // 2)
    cp_x0 = in_copy(0, x_hbm.at[first], x_ref.at[first])
    cp_w = [in_copy(1 + j, wqkv_hbm.at[:, pl.ds(j * D, D)], wqkv_ref.at[:, pl.ds(j * D, D)]) for j in range(3)]
    cp_x1 = in_copy(4, x_hbm.at[rest], x_ref.at[rest])
    cp_ffn = [in_copy(5, wo_hbm, wo_ref), in_copy(6, wg_hbm, wg_ref), in_copy(7, wu_hbm, wu_ref),
              in_copy(8, wd_hbm, wd_ref)]

    def out_copy(i, n=None):
        rows = _ds(i * TB, TB, TB)
        if n is None:
            return pltpu.make_async_copy(out_ref.at[rows], out_hbm.at[rows], out_sems.at[i])
        cols = pl.ds(n * LANES, LANES)
        return pltpu.make_async_copy(out_ref.at[rows, cols], out_hbm.at[rows, cols], out_sems.at[i + n])

    def ln1(i):
        half = pl.ds(i * (TB // 2), TB // 2)
        xn_ref[...] = _pack(_layernorm(_unpack(x_ref[half, :])))

    def norm_operands(dst_ref, r, top, bottom):
        k = D // 2
        top, bottom = _layernorm(top), _layernorm(bottom)
        for j, v in enumerate(_lhs_operands(top[:, :k], top[:, k:], bottom[:, :k], bottom[:, k:])):
            dst_ref[j, pl.ds(r // 2, 8), :] = _pack(v)

    def ln1_split(i, r, after):
        top, bottom = (_unpack(_behind(x_ref[pl.ds((i * TB + t + r) // 2, 8), :], after)) for t in (0, TB // 2))
        norm_operands(xs_ref.at[i % 2], r, top, bottom)

    def emit_qkv(y, tok0, c):
        j, n = divmod(c, D // LANES)
        rows = pl.ds(tok0 // 2, y.shape[0] // 2)
        cols = pl.ds(n * LANES, LANES)
        if j == 0:
            q_ref[rows, cols] = _bits((y * scale).astype(BF16))
        elif j == 1:
            k_ref[rows, cols] = _bits(y.astype(BF16))
        else:
            vt_ref[pl.ds(n * LANES // 2, LANES // 2), pl.ds(tok0, y.shape[0])] = _bits(_bf16(_pack(y)).T)

    def qkv(i, c):
        y = _dot(_bf16(xn_ref[...]), _bf16(wqkv_ref[:, pl.ds(c * LANES, LANES)]))
        emit_qkv(y, i * TB, c)
        return y

    def qkv_finish(i, c, prods):
        for q, y in enumerate(_combine(prods)):
            emit_qkv(y, i * TB + (q // 2) * (TB // 2), c + (q % 2) * (3 * D // 2 // LANES))

    def proj(i, n):
        half = _ds(i * (TB // 2), TB // 2, TB // 2)
        cols = pl.ds(n * LANES, LANES)
        h_ref[n, _ds(i * TB, TB, TB), :] = (
            _bf16(x_ref[half, cols]).astype(F32) + _dot(_bf16(o_ref[half, :]), _bf16(wo_ref[:, cols])))

    def ln2(i):
        def rows(r):
            return jnp.concatenate(
                [jnp.concatenate([h_ref[n, pl.ds(i * TB + r + k, 8, stride=2), :] for k in range(2)], axis=0)
                 for n in range(D // LANES)], axis=1)
        for r in range(0, TB // 2, 16):
            norm_operands(hn_ref, r, rows(r), rows(TB // 2 + r))

    def prep(w_ref, s_ref, r0, rows, c0, cols, after, factor=1.0):
        k, n = w_ref.shape[0] // 2, w_ref.shape[1] // 2
        for r in range(r0, r0 + rows, 8):
            quad = [w_ref[pl.ds(a * k + r, 8), pl.ds(b * n + c0, cols)] for a in range(2) for b in range(2)]
            quad[0], quad[3] = _behind(quad[0], after), _behind(quad[3], after)
            halves = []
            for index in range(2):
                vals = [pltpu.unpack_elementwise(v, index=index, packed_dtype=BF16, unpacked_dtype=F32)
                        for v in quad]
                if factor != 1.0:
                    vals = [v * factor for v in vals]
                halves.append(_rhs_operands(*vals))
            for j in range(7):
                if factor != 1.0 or j not in (1, 4):
                    s_ref[j, pl.ds(r, 8), pl.ds(c0, cols)] = pltpu.pack_elementwise(
                        [halves[0][j], halves[1][j]], packed_dtype=BF16).astype(U32)

    def rhs(w_ref, s_ref, j, c):
        k, n = w_ref.shape[0] // 2, w_ref.shape[1] // 2
        if j in (1, 4):
            return _bf16(w_ref[pl.ds(j // 4 * k, k), pl.ds(j // 4 * n + c * LANES, LANES)])
        return _bf16(s_ref[j, :, pl.ds(c * LANES, LANES)])

    def up_product(op, c, j):
        w = _bf16(sg_ref[j, :, pl.ds(c * LANES, LANES)]) if op == "g" else rhs(wu_ref, su_ref, j, c)
        return _dot(_bf16(hn_ref[j]), w)

    def activate(c, g, u):
        a = [(gq + gq * jnp.tanh(gq)) * uq for gq, uq in zip(g, u)]
        for j, v in enumerate(_lhs_operands(*a)):
            a_ref[j, :, pl.ds(c * LANES, LANES)] = _pack(v)

    def down_product(n, j):
        return _dot(_bf16(a_ref[j]), rhs(wd_ref, sd_ref, j, n))

    def down_finish(i, n, prods):
        m = TB // 2
        for q, y in enumerate(_combine(prods)):
            rows = _ds(i * TB + (q // 2) * m, m, m)
            cols = pl.ds((q % 2) * (D // 2) + n * LANES, LANES)
            y_ref[n, q] = y
            y = jnp.concatenate([y_ref[n, q, pl.ds(r + k, 8, stride=2), :]
                                 for r in range(0, m, 16) for k in range(2)], axis=0)
            out_ref[rows, cols] = (h_ref[(q % 2) * 2 + n, rows, :] + y).astype(out_ref.dtype)

    copies = [cp_x0] + cp_w + [cp_x1] + cp_ffn

    def run(prog, i):
        sts, pts, rs, res, prods, ups, hs = {}, {}, {}, {}, {}, {}, []
        latest = None
        for op, *args in prog:
            if op in "QSPO":
                g = args[0]
                tok0 = i * TB + (g // 4) * QBLK
                slab = g % 4
                skip = max(0, (W - tok0) // 16) if isinstance(tok0, int) else 0
                which = range(args[1], args[2]) if len(args) > 1 else range(8)
            if op == "Q":
                for t, st in zip(which, _scores(q_ref, k_ref, tok0, skip, slab, G, which)):
                    sts[g] = sts.get(g, []) + [_merge(st, skip, t % G, G, s_ref.at[g % NS, t] if NS else None)]
            elif op == "S":
                for t in which:
                    tile, total = _softmax(sts[g][t], skip, t % G, G, GPV, p_ref.at[g % NP, t] if NP else None)
                    pts[g] = pts.get(g, []) + [tile]
                    rs[g] = rs.get(g, []) + [total]
            elif op == "P":
                res[g] = res.get(g, []) + [
                    _pv(_unskew(pts[g][h // G * G:h // G * G + G], h % G, skip, G, GPV), vt_ref, tok0, skip, slab, h, G, GPV)
                    for h in which]
            elif op == "O":
                _finish(res.pop(g), rs.pop(g), o_ref, tok0, slab, G, GPV)
            elif op == "l":
                ln1(i + args[0])
            elif op == "L":
                ln1_split(args[0], args[1], latest)
            elif op == "a":
                latest = qkv(*args)
            elif op == "A":
                b, c, j = args
                ups[op] = ups.get(op, []) + [
                    _dot(_bf16(xs_ref[b % 2, j]), rhs(wqkv_ref, sq_ref, j, c))]
                latest = ups[op][-1]
                if len(ups[op]) == 7:
                    qkv_finish(b, c, ups.pop(op))
            elif op == "w":
                proj(i + args[0], args[1])
                if args[1] == D // LANES - 1:
                    ln2(i + args[0])
            elif op in "gu":
                c, j = args
                ups[op] = ups.get(op, []) + [up_product(op, c, j)]
                if len(ups[op]) == 7:
                    ups[op] = _combine(ups[op])
                    if op == "u":
                        activate(c, ups.pop("g"), ups.pop("u"))
            elif op == "d":
                b, n = args[:2]
                prods[n] = prods.get(n, []) + [down_product(n, j) for j in range(args[2], args[3])]
                if len(prods[n]) == 7:
                    down_finish(i + b, n, prods.pop(n))
            elif op == "T":
                m, c, part, parts = args
                if m == 2:
                    prep(wd_ref, sd_ref, c * 64 + part * 64 // parts, 64 // parts, 0, D // 2, latest)
                else:
                    w_ref, s_ref = ((wg_ref, sg_ref), (wu_ref, su_ref), None, (wqkv_ref, sq_ref))[m]
                    prep(w_ref, s_ref, part * D // 4 // parts, D // 4 // parts, c * LANES, LANES,
                         latest, 0.5 if m == 0 else 1.0)
            elif op == "D":
                for n in args:
                    copies[n].start()
            elif op == "W":
                for n in args:
                    copies[n].wait()
            elif op == "X":
                out_copy(i + args[0], *args[1:]).start()

    prog0, lo, hi, body, prog9 = program
    run(prog0, 0)
    if hi > lo:
        def steady(i, carry):
            run(body, i)
            return carry
        lax.fori_loop(lo, hi, steady, 0)
    run(prog9, 0)
    started = [st[1:] for st in prog0 + prog9 if st[0] == 'X'] + [(i + st[1],) for i in range(lo, hi) for st in body if st[0] == 'X']
    for i in started:
        out_copy(*i).wait()


def _cost(step):
    return {"a": 256, "w": 256, "g": 64, "u": 64, "A": 64}.get(step[0], 224 if step[0] == "d" else 0)


def _weave(dense, groups, first, last, lag, nq, np_):
    total = sum(_cost(s) for s in dense)
    period = total * (last - first) / (len(groups) + lag)
    events = []
    for k, g in enumerate(groups):
        t = total * first + k * period
        for p in range(nq):
            rng = (8 * p // nq, 8 * (p + 1) // nq)
            events.append((t + p * period / nq, 0, [("Q", g) + rng, ("S", g) + rng]))
        for p in range(np_):
            tail = [("O", g)] if p == np_ - 1 else []
            events.append((t + (lag + p / np_) * period, 1, [("P", g, 8 * p // np_, 8 * (p + 1) // np_)] + tail))
    events.sort(key=lambda e: e[:2])
    out, t = [], 0
    for s in dense:
        while events and _cost(s) and events[0][0] <= t + _cost(s) / 2:
            out += events.pop(0)[2]
        out.append(s)
        t += _cost(s)
    for e in events:
        out += e[2]
    return out


def _up():
    return [(op, c, j) for c in range(7) for op in "gu" for j in range(7)]


def _down(b):
    return [("d", b, n, j, j + 1) for n in range(2) for j in range(7)]


def _ffn(b, wpos):
    down = _down(b - 1)
    return down[:wpos] + [("w", b, n) for n in range(4)] + down[wpos:] + _up()


def _spread(steps, extra):
    out, left = [], list(extra)
    for n, step in enumerate(steps):
        out.append(step)
        while left and (len(extra) - len(left)) * len(steps) < (n + 1) * len(extra):
            out.append(left.pop(0))
    return out


def build(NB=8, p0=(0.03, 0.4, 1.0, 8, 8), p1=(0.0, 0.97, 1.0, 8, 8), tpos=130, wpos=12, nhi=8, mode=1, wback=14,
          lspan=32, std=1, tend=14):
    def a(b):
        return [("a", b, c) for c in range(12)]

    def ln(b):
        return [("L", b, r) for r in range(0, 128, 16)]
    first = a(0)
    prep3 = [("T", 3, c, p, 4) for c in range(6) for p in range(4)]
    start = [("D", 0, 1, 2, 3, 4), ("W", 0), ("l", 0), ("W", 1), ("D", 5, 6, 7, 8)] + first[:4] + [("W", 2, 3, 4)]
    if std == 1:
        start += _spread(first[4:], _spread(prep3, ln(1)))
    else:
        start += _spread(first[4:], prep3[:12]) + [("l", 1)] + _spread(a(1), _spread(prep3[12:], ln(2)))
    dense = []
    for b in range(std, NB):
        steps = [("A", b, c, j) for c in range(6) for j in range(7)]
        dense += _spread(steps[:lspan], ln(b + 1) if b + 1 < NB else []) + steps[lspan:]
    preps = [("T", m, c, p, 8) for m in range(3) for c in range(7) for p in range(8)]
    dense = dense[:tpos] + [("W", 5, 6, 7, 8)] + _spread(dense[tpos:-tend], preps) + dense[-tend:]
    dense = dense[:-wback] + [("w", 0, n) for n in range(4)] + dense[-wback:]
    down = _down(NB - 1)
    tail = down[:7] + [("X", NB - 1, 0), ("X", NB - 1, 2)] + down[7:] + [("X", NB - 1, 1), ("X", NB - 1, 3)]
    if mode == 0:
        prog0 = start + _weave(dense + _up(), list(range(16)), *p0)
        body = _weave(_ffn(-1, wpos), list(range(8)), *p1) + [("X", -2)]
        return prog0, 2, nhi, body, _ffn(NB - 1, wpos) + [("X", NB - 2)] + tail
    prog0 = start + _weave(dense, list(range(8)), *p0)
    down = _down(-1)
    head = _weave(_up() + down[:wpos], list(range(8)), *p1)
    return prog0, 1, nhi, head + [("w", 0, n) for n in range(4)] + down[wpos:] + [("X", -1)], _up() + tail


def make(TB=256, G=8, GPV=2, NP=3, NS=0, NG=0, flags=None, **kw):
    program = build(**kw)

    def run(A_x, A_wqkv, A_wo, B_x, B_w_gate, B_w_up, B_w_down):
        B, S, D = A_x.shape
        F = B_w_gate.shape[1]
        hbm = pl.BlockSpec(memory_space=pl.ANY)
        out = pl.pallas_call(
            functools.partial(_kernel, TB=TB, G=G, GPV=GPV, NP=NP, NS=NS, NG=NG, program=program),
            in_specs=[hbm] * 6,
            out_specs=hbm,
            out_shape=jax.ShapeDtypeStruct((S, D), A_x.dtype),
            scratch_shapes=[
                pltpu.VMEM((S // 2, D), U32),
                pltpu.VMEM((D // 2, 3 * D), U32), pltpu.VMEM((D // 2, D), U32),
                pltpu.VMEM((D // 2, F), U32), pltpu.VMEM((D // 2, F), U32), pltpu.VMEM((F // 2, D), U32),
                pltpu.VMEM((S, D), BF16),
                pltpu.VMEM((TB // 2, D), U32),
                pltpu.VMEM((S // 2, D), U32), pltpu.VMEM((S // 2, D), U32), pltpu.VMEM((D // 2, S), U32),
                pltpu.VMEM((S // 2, D), U32),
                pltpu.VMEM((D // LANES, S, LANES), F32), pltpu.VMEM((7, TB // 4, D // 2), U32), pltpu.VMEM((7, TB // 4, F // 2), U32),
                pltpu.VMEM((7, D // 4, F // 2), U32), pltpu.VMEM((7, D // 4, F // 2), U32),
                pltpu.VMEM((7, F // 4, D // 2), U32),
                pltpu.VMEM((max(NP, 1), 8, (W + QBLK // G) // 2, LANES), U32),
                pltpu.VMEM((2, 4, TB // 2, LANES), F32),
                pltpu.VMEM((max(NS, 1), 8, W, LANES), F32), pltpu.VMEM((2, 7, TB // 4, D // 2), U32), pltpu.VMEM((7, D // 4, 3 * D // 2), U32),
                pltpu.SemaphoreType.DMA((9,)), pltpu.SemaphoreType.DMA((S // TB + 3,)),
            ],
            compiler_params=pltpu.CompilerParams(vmem_limit_bytes=100 * 2**20, flags=flags),
        )(A_x.reshape(S, D), A_wqkv, A_wo, B_w_gate, B_w_up, B_w_down)
        return out.reshape(B, S, D)
    return jax.jit(run)


pallas_sequential_preLN__sliding_block__swiglu_ffn__prompt_kernel = make()
```

```python
import math

import jax
import jax.numpy as jnp
from jax import lax
import jax.experimental.pallas as pl
import jax.experimental.pallas.tpu as pltpu

DH = 16
W = 256
LANES = 128
QBLK = 128
TB = 256
NP = 3
EPS = 1e-5
BF16 = jnp.bfloat16
F32 = jnp.float32
U32 = jnp.uint32


def _bits(x):
    return pltpu.bitcast(x, U32)


def _bf16(x):
    return pltpu.bitcast(x, BF16)


def _pack(x):
    return jnp.concatenate(
        [pltpu.pack_elementwise([x[r:r + 8], x[r + 8:r + 16]], packed_dtype=BF16).astype(U32)
         for r in range(0, x.shape[0], 16)], axis=0)


def _unpack(w):
    return jnp.concatenate(
        [pltpu.unpack_elementwise(w[r:r + 8], index=k, packed_dtype=BF16, unpacked_dtype=F32)
         for r in range(0, w.shape[0], 8) for k in range(2)], axis=0)


def _dot(a, b):
    return jnp.dot(a, b, preferred_element_type=F32)


def _layernorm(x):
    m = jnp.mean(x, axis=-1, keepdims=True)
    c = x - m
    v = jnp.mean(c * c, axis=-1, keepdims=True)
    return c * lax.rsqrt(v + EPS)


def _sel(mask, a, b):
    if a is None and b is None:
        return None
    if a is None:
        a = jnp.zeros_like(b)
    if b is None:
        b = jnp.zeros_like(a)
    return jnp.where(mask, a, b)


def _ds(start, size, align):
    if isinstance(start, int):
        return pl.ds(start, size)
    return pl.ds(pl.multiple_of(start, align), size)


def _key_range(s, skip):
    return max(s, skip), s + 17


def _edge_mask():
    key = lax.broadcasted_iota(jnp.int32, (16, LANES), 0)
    query = lax.broadcasted_iota(jnp.int32, (16, LANES), 1) & 15
    return key > query


def _scores(q_ref, k_ref, tok0, skip, slab, s):
    lanes = pl.ds(slab * LANES, LANES)
    head = lax.broadcasted_iota(jnp.int32, (8, LANES), 1) // DH
    half0 = tok0 // 2
    qs = q_ref[_ds(half0 + 8 * s, 8, 8), lanes]
    qbd = _bf16(jnp.concatenate([jnp.where(head == p ^ s, qs, jnp.zeros_like(qs)) for p in range(8)], axis=0))
    lo, hi = _key_range(s, skip)
    keys = _bf16(k_ref[_ds(half0 - W // 2 + 8 * lo, 8 * (hi - lo), 8), lanes])
    st = lax.dot_general(keys, qbd, (((1,), (1,)), ((), ())), preferred_element_type=F32)
    n = st.shape[0]
    if lo == s:
        parts = [st[16:n - 16], jnp.where(_edge_mask(), st[:16], st[n - 16:])]
    else:
        parts = [st[:n - 16]] if n > 16 else []
        parts.append(jnp.where(_edge_mask(), -1e30, st[n - 16:]))
    st = jnp.concatenate(parts, axis=0)
    return st, jnp.max(st, axis=0, keepdims=True)


def _softmax(st, m, skip, s, p_ref):
    p = jnp.exp2(st - m)
    total = jnp.broadcast_to(jnp.sum(p, axis=0, keepdims=True), (8, LANES))
    n = st.shape[0] - 16
    parts = [jnp.where(_edge_mask(), p[n:], 0.0)] if s >= skip else []
    parts += [p[:n]] if n else []
    parts += [jnp.where(_edge_mask(), 0.0, p[n:])]
    packed = _pack(jnp.concatenate(parts, axis=0))
    p_ref[pl.ds(0, packed.shape[0]), :] = packed
    return total


def _pv(p_ref, vt_ref, tok0, skip, slab, t):
    lane = lax.broadcasted_iota(jnp.int32, (8, LANES), 1)

    def pick(t, k, w):
        if k == 0:
            lo, hi = _key_range(t, skip)
            return p_ref[t, pl.ds(8 * (w - lo), 8), :] if lo <= w < hi else None
        bit = ((lane // 16) >> (k - 1)) & 1 == 1
        return _sel(bit, pick(t ^ (1 << (k - 1)), k - 1, w), pick(t, k - 1, w))
    w0 = skip // 8 * 8
    rows = [pick(t, 2, w) for w in range(w0, 24)]
    pt = _bf16(jnp.concatenate([x if x is not None else jnp.zeros((8, LANES), U32) for x in rows], axis=0))
    keys = _ds(tok0 - W + 16 * w0, 16 * (24 - w0), LANES)
    v = jnp.concatenate([vt_ref[pl.ds((slab * 8 + h) * 8, 8), keys] for h in (t, t ^ 4)], axis=0)
    return _dot(_bf16(v), pt)


def _finish(res, sums, o_ref, tok0, slab):
    lane = lax.broadcasted_iota(jnp.int32, (8, LANES), 1)
    row = lax.broadcasted_iota(jnp.int32, (8, LANES), 0)
    for k in range(3):
        bit = ((lane // 16) >> k) & 1 == 1
        sums = [jnp.where(bit, sums[t ^ (1 << k)], sums[t]) for t in range(8)]
    inv = sums[0]
    for t in range(1, 8):
        inv = jnp.where(row == t, sums[t], inv)
    inv = 1.0 / inv
    outs = []
    for h in range(8):
        scale = jnp.broadcast_to(inv[h:h + 1], (8, LANES))
        outs += [jnp.where(lane < 64, res[h][:8], res[h ^ 4][16:24]) * scale,
                 jnp.where(lane < 64, res[h][8:16], res[h ^ 4][24:]) * scale]
    o = _bits(jnp.concatenate(outs, axis=0).astype(BF16).T)
    parts = [o[8 * p:8 * p + 8] for p in range(8)]
    for k in range(3):
        bit = ((lane // DH) >> k) & 1 == 1
        parts = [jnp.where(bit, parts[p ^ (1 << k)], parts[p]) for p in range(8)]
    o_ref[_ds(tok0 // 2, QBLK // 2, 8), pl.ds(slab * LANES, LANES)] = jnp.concatenate(parts, axis=0)


def _behind(words, after):
    if after is None:
        return words
    lane = lax.broadcasted_iota(jnp.int32, words.shape, 1)
    never = (lane * lane) & 2 != 0
    anchor = jnp.concatenate([pltpu.bitcast(after[:8], U32)] * (words.shape[1] // LANES), axis=1)
    return jnp.where(never, anchor, words)


def _lhs_operands(a11, a12, a21, a22):
    return [a11 + a22, a21 + a22, a11, a22, a11 + a12, a21 - a11, a12 - a22]


def _rhs_operands(b11, b12, b21, b22):
    return [b11 + b22, b11, b12 - b22, b21 - b11, b22, b11 + b12, b21 + b22]


def _combine(m):
    return (m[0] + m[3]) + (m[6] - m[4]), m[2] + m[4], m[1] + m[3], (m[0] - m[1]) + (m[2] + m[5])


def _kernel(x_hbm, wqkv_hbm, wo_hbm, wg_hbm, wu_hbm, wd_hbm, out_hbm,
            x_ref, wqkv_ref, wo_ref, wg_ref, wu_ref, wd_ref, out_ref,
            xn_ref, q_ref, k_ref, vt_ref, o_ref, h_ref, hn_ref, a_ref, sg_ref, su_ref, sd_ref, p_ref, xs_ref, sq_ref, in_sems, out_sems):
    S, D = out_ref.shape
    F = wg_ref.shape[-1]
    NB = S // TB
    scale = DH ** -0.5 * math.log2(math.e)

    def in_copy(n, src, dst):
        return pltpu.make_async_copy(src, dst, in_sems.at[n])

    x_hbm, wqkv_hbm, wo_hbm, wg_hbm, wu_hbm, wd_hbm = (r.bitcast(U32) for r in (x_hbm, wqkv_hbm, wo_hbm, wg_hbm, wu_hbm, wd_hbm))
    first = pl.ds(0, TB // 2)
    second = pl.ds(TB // 2, TB // 2)
    rest = pl.ds(TB, S // 2 - TB)
    cp_x0 = in_copy(0, x_hbm.at[first], x_ref.at[first])
    cp_w = [in_copy(1 + j, wqkv_hbm.at[:, pl.ds(j * D, D)], wqkv_ref.at[:, pl.ds(j * D, D)]) for j in range(3)]
    cp_x1 = in_copy(4, x_hbm.at[rest], x_ref.at[rest])
    cp_ffn = [in_copy(5, wo_hbm, wo_ref), in_copy(6, wg_hbm, wg_ref), in_copy(7, wu_hbm, wu_ref),
              in_copy(8, wd_hbm, wd_ref)]

    def out_copy(i, n=None):
        rows = _ds(i * TB, TB, TB)
        if n is None:
            return pltpu.make_async_copy(out_ref.at[rows], out_hbm.at[rows], out_sems.at[i])
        cols = pl.ds(n * LANES, LANES)
        return pltpu.make_async_copy(out_ref.at[rows, cols], out_hbm.at[rows, cols], out_sems.at[i + n])

    def ln1(i):
        half = pl.ds(i * (TB // 2), TB // 2)
        xn_ref[...] = _pack(_layernorm(_unpack(x_ref[half, :])))

    def norm_operands(dst_ref, r, top, bottom):
        k = D // 2
        top, bottom = _layernorm(top), _layernorm(bottom)
        for j, v in enumerate(_lhs_operands(top[:, :k], top[:, k:], bottom[:, :k], bottom[:, k:])):
            dst_ref[j, pl.ds(r // 2, 8), :] = _pack(v)

    def ln1_split(i, r, after):
        top, bottom = (_unpack(_behind(x_ref[pl.ds((i * TB + t + r) // 2, 8), :], after)) for t in (0, TB // 2))
        norm_operands(xs_ref.at[i % 2], r, top, bottom)

    def emit_qkv(y, tok0, c):
        j, n = divmod(c, D // LANES)
        rows = pl.ds(tok0 // 2, y.shape[0] // 2)
        cols = pl.ds(n * LANES, LANES)
        if j == 0:
            q_ref[rows, cols] = _bits((y * scale).astype(BF16))
        elif j == 1:
            k_ref[rows, cols] = _bits(y.astype(BF16))
        else:
            vt_ref[pl.ds(n * LANES // 2, LANES // 2), pl.ds(tok0, y.shape[0])] = _bits(_bf16(_pack(y)).T)

    def qkv(i, c):
        y = _dot(_bf16(xn_ref[...]), _bf16(wqkv_ref[:, pl.ds(c * LANES, LANES)]))
        emit_qkv(y, i * TB, c)
        return y

    def qkv_finish(i, c, prods):
        for q, y in enumerate(_combine(prods)):
            emit_qkv(y, i * TB + (q // 2) * (TB // 2), c + (q % 2) * (3 * D // 2 // LANES))

    def proj(i, n):
        half = _ds(i * (TB // 2), TB // 2, TB // 2)
        cols = pl.ds(n * LANES, LANES)
        h_ref[n, _ds(i * TB, TB, TB), :] = (
            _bf16(x_ref[half, cols]).astype(F32) + _dot(_bf16(o_ref[half, :]), _bf16(wo_ref[:, cols])))

    def ln2(i):
        def rows(r):
            return jnp.concatenate([h_ref[n, _ds(i * TB + r, 16, 16), :] for n in range(D // LANES)], axis=1)
        for r in range(0, TB // 2, 16):
            norm_operands(hn_ref, r, rows(r), rows(TB // 2 + r))

    def prep(w_ref, s_ref, r0, rows, c0, cols, after, factor=1.0):
        k, n = w_ref.shape[0] // 2, w_ref.shape[1] // 2
        for r in range(r0, r0 + rows, 8):
            quad = [w_ref[pl.ds(a * k + r, 8), pl.ds(b * n + c0, cols)] for a in range(2) for b in range(2)]
            quad[0], quad[3] = _behind(quad[0], after), _behind(quad[3], after)
            halves = []
            for index in range(2):
                vals = [pltpu.unpack_elementwise(v, index=index, packed_dtype=BF16, unpacked_dtype=F32)
                        for v in quad]
                if factor != 1.0:
                    vals = [v * factor for v in vals]
                halves.append(_rhs_operands(*vals))
            for j in range(7):
                if factor != 1.0 or j not in (1, 4):
                    s_ref[j, pl.ds(r, 8), pl.ds(c0, cols)] = pltpu.pack_elementwise(
                        [halves[0][j], halves[1][j]], packed_dtype=BF16).astype(U32)

    def rhs(w_ref, s_ref, j, c):
        k, n = w_ref.shape[0] // 2, w_ref.shape[1] // 2
        if j in (1, 4):
            return _bf16(w_ref[pl.ds(j // 4 * k, k), pl.ds(j // 4 * n + c * LANES, LANES)])
        return _bf16(s_ref[j, :, pl.ds(c * LANES, LANES)])

    def up_product(op, c, j):
        w = _bf16(sg_ref[j, :, pl.ds(c * LANES, LANES)]) if op == "gate" else rhs(wu_ref, su_ref, j, c)
        return _dot(_bf16(hn_ref[j]), w)

    def activate(c, g, u):
        a = [(gq + gq * jnp.tanh(gq)) * uq for gq, uq in zip(g, u)]
        for j, v in enumerate(_lhs_operands(*a)):
            a_ref[j, :, pl.ds(c * LANES, LANES)] = _pack(v)

    def down_product(n, j):
        return _dot(_bf16(a_ref[j]), rhs(wd_ref, sd_ref, j, n))

    def down_finish(i, n, prods):
        m = TB // 2
        for q, y in enumerate(_combine(prods)):
            rows = _ds(i * TB + (q // 2) * m, m, m)
            cols = pl.ds((q % 2) * (D // 2) + n * LANES, LANES)
            for _ in range(2):
                y = _bf16(_pack(y)).astype(F32)
            out_ref[rows, cols] = (h_ref[(q % 2) * 2 + n, rows, :] + y).astype(out_ref.dtype)

    copies = [cp_x0] + cp_w + [cp_x1] + cp_ffn + [in_copy(9, x_hbm.at[second], x_ref.at[second])]

    def run(prog, i):
        sums, res, prods, latest = {}, {}, {}, None
        for op, *args in prog:
            if op in ("score", "pv", "finish"):
                g = args[0]
                tok0 = i * TB + (g // 4) * QBLK
                slab = g % 4
                skip = max(0, (W - tok0) // 16) if isinstance(tok0, int) else 0
            if op == "score":
                st, m = _scores(q_ref, k_ref, tok0, skip, slab, args[1])
                sums.setdefault(g, []).append(_softmax(st, m, skip, args[1], p_ref.at[g % NP, args[1]]))
            elif op == "pv":
                res.setdefault(g, {})[args[1]] = _pv(p_ref.at[g % NP], vt_ref, tok0, skip, slab, args[1])
            elif op == "finish":
                _finish(res.pop(g), sums.pop(g), o_ref, tok0, slab)
            elif op == "ln1":
                ln1(args[0])
            elif op == "ln1_split":
                ln1_split(args[0], args[1], latest)
            elif op == "qkv":
                latest = qkv(*args)
            elif op == "qkv_product":
                b, c, j = args
                latest = _dot(_bf16(xs_ref[b % 2, j]), rhs(wqkv_ref, sq_ref, j, c))
                prods.setdefault(op, []).append(latest)
                if j == 6:
                    qkv_finish(b, c, prods.pop(op))
            elif op == "proj":
                proj(i, args[0])
                if args[0] == D // LANES - 1:
                    ln2(i)
            elif op in ("gate", "up"):
                c, j = args
                prods.setdefault(op, []).append(up_product(op, c, j))
                if j == 6:
                    prods[op] = _combine(prods[op])
                    if op == "up":
                        activate(c, prods.pop("gate"), prods.pop("up"))
            elif op == "down":
                b, n, j = args
                prods.setdefault(op, []).append(down_product(n, j))
                if j == 6:
                    down_finish(i + b, n, prods.pop(op))
            elif op == "prep":
                name, c, part, parts = args
                if name == "down":
                    prep(wd_ref, sd_ref, c * 64 + part * 64 // parts, 64 // parts, 0, D // 2, latest)
                else:
                    w_ref, s_ref = {"gate": (wg_ref, sg_ref), "up": (wu_ref, su_ref), "qkv": (wqkv_ref, sq_ref)}[name]
                    prep(w_ref, s_ref, part * D // 4 // parts, D // 4 // parts, c * LANES, LANES, latest,
                         0.5 if name == "gate" else 1.0)
            elif op == "fetch":
                for n in args:
                    copies[n].start()
            elif op == "wait":
                for n in args:
                    copies[n].wait()
            elif op == "send":
                out_copy(i + args[0], *args[1:]).start()

    prologue, body, epilogue = _schedule(NB)
    run(prologue, 0)

    def steady(i, carry):
        run(body, i)
        return carry
    lax.fori_loop(1, NB, steady, 0)
    run(epilogue, 0)
    for i in range(NB - 1):
        out_copy(i).wait()
    for n in range(D // LANES):
        out_copy(NB - 1, n).wait()


def _cost(step):
    return {"qkv": 256, "proj": 256, "qkv_product": 64, "gate": 64, "up": 64, "down": 224}.get(step[0], 0)


def _weave(dense, first, last, lag):
    total = sum(_cost(s) for s in dense)
    period = total * (last - first) / (8 + lag)
    events = []
    for g in range(8):
        t = total * first + g * period
        for p in range(8):
            events.append((t + p * period / 8, 0, [("score", g, p)]))
        for p, h in enumerate((0, 2, 1, 3, 4, 6, 5, 7)):
            events.append((t + (lag + p / 8) * period, 1, [("pv", g, h)] + [("finish", g)] * (p == 7)))
    events.sort(key=lambda e: e[:2])
    out, t = [], 0
    for s in dense:
        while events and _cost(s) and events[0][0] <= t + _cost(s) / 2:
            out += events.pop(0)[2]
        out.append(s)
        t += _cost(s)
    for e in events:
        out += e[2]
    return out


def _spread(steps, extra):
    out, left = [], list(extra)
    for n, step in enumerate(steps):
        out.append(step)
        while left and (len(extra) - len(left)) * len(steps) < (n + 1) * len(extra):
            out.append(left.pop(0))
    return out


def _schedule(NB):
    def norm(b):
        return [("ln1_split", b, r) for r in range(0, TB // 2, 16)]

    def down(b):
        return [("down", b, n, j) for n in range(2) for j in range(7)]
    proj = [("proj", n) for n in range(4)]
    up = [(op, c, j) for c in range(7) for op in ("gate", "up") for j in range(7)]

    qkv = [("qkv", 0, c) for c in range(12)]
    prep = [("prep", "qkv", c, p, 4) for c in range(6) for p in range(4)]
    start = ([("fetch", 0, 1, 2, 9, 3, 4, 5, 6, 7, 8), ("wait", 0), ("ln1", 0), ("wait", 1)] + qkv[:4]
             + [("wait", 2, 9)] + _spread(qkv[4:8], _spread(prep[:8], norm(1)))
             + [("wait", 3)] + _spread(qkv[8:], prep[8:]))
    dense = []
    for b in range(1, NB):
        steps = [("qkv_product", b, c, j) for c in range(6) for j in range(7)]
        if b == 1:
            dense += steps[:21] + [("wait", 4)] + _spread(steps[21:-4], norm(2)) + steps[-4:]
        else:
            dense += _spread(steps[:24], norm(b + 1) if b + 1 < NB else []) + steps[24:]
    prep = [("prep", name, c, p, 8) for name in ("gate", "up", "down") for c in range(7) for p in range(8)]
    dense = dense[:185] + [("wait", 5, 6, 7, 8)] + _spread(dense[185:-14], prep) + proj + dense[-14:]
    prologue = start + _weave(dense, 0.094, 0.417, 1.2)

    body = _weave(up + down(-1)[:12], 0.0, 0.97, 1.0) + proj + down(-1)[12:] + [("send", -1)]

    last = down(NB - 1)
    epilogue = (up + last[:7] + [("send", NB - 1, 0), ("send", NB - 1, 2)]
                + last[7:] + [("send", NB - 1, 1), ("send", NB - 1, 3)])
    return prologue, body, epilogue


@jax.jit
def pallas_sequential_preLN__sliding_block__swiglu_ffn__prompt_kernel(
    A_x: jax.Array,
    A_wqkv: jax.Array,
    A_wo: jax.Array,
    B_x: jax.Array,
    B_w_gate: jax.Array,
    B_w_up: jax.Array,
    B_w_down: jax.Array,
):
    del B_x
    B, S, D = A_x.shape
    F = B_w_gate.shape[1]
    assert (B, S, D, F) == (1, 2048, 512, 1792)
    hbm = pl.BlockSpec(memory_space=pl.ANY)

    def words(*shape):
        return pltpu.VMEM(shape, U32)
    out = pl.pallas_call(
        _kernel,
        in_specs=[hbm] * 6,
        out_specs=hbm,
        out_shape=jax.ShapeDtypeStruct((S, D), A_x.dtype),
        scratch_shapes=[
            words(S // 2, D), words(D // 2, 3 * D), words(D // 2, D),
            words(D // 2, F), words(D // 2, F), words(F // 2, D),
            pltpu.VMEM((S, D), BF16),
            words(TB // 2, D),
            words(S // 2, D), words(S // 2, D), words(D // 2, S),
            words(S // 2, D), pltpu.VMEM((D // LANES, S, LANES), F32),
            words(7, TB // 4, D // 2), words(7, TB // 4, F // 2),
            words(7, D // 4, F // 2), words(7, D // 4, F // 2), words(7, F // 4, D // 2),
            words(NP, 8, (W + 16) // 2, LANES),
            words(2, 7, TB // 4, D // 2), words(7, D // 4, 3 * D // 2),
            pltpu.SemaphoreType.DMA((10,)), pltpu.SemaphoreType.DMA((S // TB + 3,)),
        ],
        compiler_params=pltpu.CompilerParams(vmem_limit_bytes=100 * 2**20),
    )(A_x.reshape(S, D), A_wqkv, A_wo, B_w_gate, B_w_up, B_w_down)
    return out.reshape(B, S, D)
```
